```python
import os as _os
_os.environ.setdefault("JAX_PLATFORMS", "cpu")
import jax
import jax.numpy as jnp

def _softmax(x, axis=-1):
    return jax.nn.softmax(x, axis=axis)
def _gelu(x):
    return jax.nn.gelu(x, approximate=True)
def _silu(x):
    return jax.nn.silu(x)
def _sigmoid(x):
    return jax.nn.sigmoid(x)
def _layernorm(x, axis=-1, eps=1e-5):
    m = jnp.mean(x, axis=axis, keepdims=True)
    v = jnp.var(x, axis=axis, keepdims=True)
    return (x - m) / jnp.sqrt(v + eps)
def _scatter_add(tgt, idx, src, axis=0):
    return tgt.at[idx].add(src)
def _segment_sum(src, seg, n):
    return jax.ops.segment_sum(src, seg, n)
class _Rng:
    def __init__(self, key):
        self._k = key
    def _next(self):
        self._k, sub = jax.random.split(self._k)
        return sub
    def normal(self, shape):
        return jax.random.normal(self._next(), shape, dtype=jnp.bfloat16)
    def randint(self, lo, hi, shape):
        return jax.random.randint(self._next(), shape, lo, hi, dtype=jnp.int32)
    def uniform(self, shape, lo=0.0, hi=1.0):
        return jax.random.uniform(self._next(), shape, jnp.bfloat16, lo, hi)
    def permutation(self, n):
        return jax.random.permutation(self._next(), n)


kernel_name = 'parallel_sum__ssm_conv_s4__mixer_channel_mlp__prompt'

def setup_inputs():
    _rng = _Rng(jax.random.key(int.from_bytes(__import__("os").urandom(4), "little")))
    _w = (lambda a: (lambda t: t.astype(jnp.bfloat16) if jnp.issubdtype(t.dtype, jnp.floating) else t)(jnp.asarray(a)))
    def _A_setup():
        B, L, D, N = 1, 2048, 512, 128
        A_re = -jnp.exp((lambda *s: _rng.normal(s) * 0.1)(D, N))
        A_im = jnp.pi * (lambda *s: _rng.normal(s) * 0.1)(D, N)
        B_re = (lambda *s: _rng.normal(s) * 0.1)(D, N)
        B_im = (lambda *s: _rng.normal(s) * 0.1)(D, N)
        C_re = (lambda *s: _rng.normal(s) * 0.1)(D, N)
        C_im = (lambda *s: _rng.normal(s) * 0.1)(D, N)
        log_dt = (lambda *s: _rng.normal(s) * 0.1)(D) * 0.5 - 4.0
        Dskip = (lambda *s: _rng.normal(s) * 0.05)(D)
        return {
            "u": _w((lambda *s: _rng.normal(s) * 0.05)(B, L, D)),
            "A_re": _w(A_re),
            "A_im": _w(A_im),
            "B_re": _w(B_re),
            "B_im": _w(B_im),
            "C_re": _w(C_re),
            "C_im": _w(C_im),
            "log_dt": _w(log_dt),
            "Dskip": _w(Dskip),
        }
    _A_in = _A_setup()

    def _B_setup():
        B, S, D, F = 1, 2048, 512, 1792
        return {
            "x": _w((lambda *s: _rng.normal(s) * 0.05)(B, S, D)),
            "w1": _w((lambda *s: _rng.normal(s) * 0.2)(D, F) * (D ** -0.5)),
            "b1": _w((lambda *s: _rng.normal(s) * 0.2)(F)),
            "w2": _w((lambda *s: _rng.normal(s) * 0.2)(F, D) * (F ** -0.5)),
            "b2": _w((lambda *s: _rng.normal(s) * 0.05)(D)),
        }
    _B_in = _B_setup()

    return {
        "A_u": _A_in["u"],
        "A_A_re": _A_in["A_re"],
        "A_A_im": _A_in["A_im"],
        "A_B_re": _A_in["B_re"],
        "A_B_im": _A_in["B_im"],
        "A_C_re": _A_in["C_re"],
        "A_C_im": _A_in["C_im"],
        "A_log_dt": _A_in["log_dt"],
        "A_Dskip": _A_in["Dskip"],
        "B_x": _B_in["x"],
        "B_w1": _B_in["w1"],
        "B_b1": _B_in["b1"],
        "B_w2": _B_in["w2"],
        "B_b2": _B_in["b2"],
    }

def reference(A_u, A_A_re, A_A_im, A_B_re, A_B_im, A_C_re, A_C_im, A_log_dt, A_Dskip, B_x, B_w1, B_b1, B_w2, B_b2):
    def _A_ref(u, A_re, A_im, B_re, B_im, C_re, C_im, log_dt, Dskip):
        Bsz, L, D = u.shape
        dt = jnp.exp(log_dt)[:, None]
        A = A_re + 1j * A_im
        Bc = B_re + 1j * B_im
        Cc = C_re + 1j * C_im
        logdA = dt * A
        dB = dt * Bc
        l = (lambda x, dt: x.astype(dt))(jnp.arange(L), A_re.dtype)
        P = jnp.exp(logdA[:, :, None] * l[None, None, :])
        K = jnp.einsum("dn,dnl,dn->dl", Cc, P, dB).real
        L2 = 2 * L
        Kp = jnp.pad(K, ((0, 0), (0, L)))
        up = (lambda x, *d: x.transpose(*d))(u, 0, 2, 1)
        up = jnp.pad(up, ((0, 0), (0, 0), (0, L)))
        Kf = (lambda x, axes=(-2,-1): jnp.fft.rfft2(x.astype(jnp.float32), axes=axes))(Kp[:, None, :], axes=(-2, -1))
        Uf = (lambda x, axes=(-2,-1): jnp.fft.rfft2(x.astype(jnp.float32), axes=axes))(up[:, :, None, :], axes=(-2, -1))
        Yf = Uf * Kf[None, :, :, :]
        y = (lambda x, s, axes=(-2,-1): jnp.fft.irfft2(x, s=s, axes=axes).astype(jnp.bfloat16))(Yf, (1, L2), axes=(-2, -1))[:, :, 0, :L]
        y = (lambda x, *d: x.transpose(*d))(y, 0, 2, 1) + u * Dskip[None, None, :]
        return y

    def _B_ref(x, w1, b1, w2, b2):
        y = _layernorm(x, axis=-1)
        h = _gelu(jnp.einsum("bsd,df->bsf", y, w1) + b1)
        return jnp.einsum("bsf,fd->bsd", h, w2) + b2

    x = A_u
    xn = _layernorm(x, axis=-1)
    return x + _A_ref(xn, A_A_re, A_A_im, A_B_re, A_B_im, A_C_re, A_C_im, A_log_dt, A_Dskip) + _B_ref(xn, B_w1, B_b1, B_w2, B_b2)
```

```python
import functools
import numpy as np
import jax
import jax.numpy as jnp
from jax import lax
import jax.experimental.pallas as pl
import jax.experimental.pallas.tpu as pltpu

f32 = jnp.float32
bf16 = jnp.bfloat16
i32 = jnp.int32

L = 2048
D = 512
N = 128
F = 1792
P = 128
NB = L // P
FR = 264
RE_ROWS = 136
MB = 256
MERGE = False


def _r(x):
    return x.astype(bf16).astype(f32)


def _ln(xf):
    mean = jnp.mean(xf, axis=-1, keepdims=True)
    cen = xf - mean
    var = jnp.mean(cen * cen, axis=-1, keepdims=True)
    m_b = _r(mean)
    v_b = _r(var)
    d = _r(xf - m_b)
    den = _r(jnp.sqrt(_r(v_b + 1e-5)))
    return _r(d / den)


def _split2(a):
    hi = a.astype(bf16)
    lo = (a - hi.astype(f32)).astype(bf16)
    return hi, lo


def _dot(a, b):
    return jnp.dot(a, b, preferred_element_type=f32)


def _dft_rows(delta):
    kk = lax.broadcasted_iota(i32, (FR, P), 0)
    is_re = kk < RE_ROWS
    kfreq = jnp.where(is_re, kk, kk - RE_ROWS)
    valid = jnp.logical_or(jnp.logical_not(is_re), kk <= P)
    ang = ((kfreq * delta) % (2 * P)).astype(f32) * f32(np.pi / P)
    Rm = jnp.where(is_re, jnp.cos(ang), -jnp.sin(ang))
    return jnp.where(valid, Rm, 0.0)


def kernel(x_hbm, are_ref, aim_ref, bre_ref, bim_ref, cre_ref, cim_ref, ldt_ref, dsk_ref,
           w1_hbm, b1_ref, w2_hbm, b2_ref, o_hbm,
           xr_s, xi_s, yr_s, yi_s, g_s, kh_s, v_s, rhi_s, rlo_s, ihi_s, ilo_s, xn_s, w_s,
           x_s, w1_s, w2_s, yn_s, h_s, yb_s, o_s, sems):
    cp_x = pltpu.make_async_copy(x_hbm, x_s, sems.at[0])
    cp_w1 = pltpu.make_async_copy(w1_hbm, w1_s, sems.at[1])
    cp_w2 = pltpu.make_async_copy(w2_hbm, w2_s, sems.at[2])
    cp_x.start()
    cp_w1.start()
    cp_w2.start()

    with jax.named_scope('dftmat'):
        jj = lax.broadcasted_iota(i32, (FR, P), 1)
        Rm = _dft_rows(jj)
        ii = lax.broadcasted_iota(i32, (P, FR), 0)
        kc = lax.broadcasted_iota(i32, (P, FR), 1)
        c_re = kc < RE_ROWS
        kf2 = jnp.where(c_re, kc, kc - RE_ROWS)
        ang2 = ((kf2 * ii) % (2 * P)).astype(f32) * f32(np.pi / P)
        wgt = jnp.where((kf2 == 0) | (kf2 == P), 1.0, 2.0) * f32(1.0 / (2 * P))
        valid2 = jnp.logical_or(jnp.logical_not(c_re), kc <= P)
        Im = jnp.where(c_re, jnp.cos(ang2), -jnp.sin(ang2)) * wgt
        Im = jnp.where(valid2, Im, 0.0)
        ih, il = _split2(Im)
        ihi_s[...] = ih
        ilo_s[...] = il
        h, l_ = _split2(Rm)
        rhi_s[0] = h
        rlo_s[0] = l_
        rho = jj
        delta_near = 64 * (rho // 64) + 16 * ((rho // 4) % 4) + 4 * ((rho // 16) % 4) + rho % 4
        h, l_ = _split2(_dft_rows(delta_near))
        rhi_s[1] = h
        rlo_s[1] = l_
        r_hi = Rm.astype(bf16)
        rem1 = Rm - r_hi.astype(f32)
        r_mid = rem1.astype(bf16)
        r_lo = (rem1 - r_mid.astype(f32)).astype(bf16)
        dl = lax.broadcasted_iota(i32, (P, P), 0)
        col = lax.broadcasted_iota(i32, (P, P), 1)
        for vi, (r, woff) in enumerate([(1, 0), (2, 0), (3, 0), (3, 8)]):
            s = 1 << r
            fl = dl >> r
            rem = dl & (s - 1)
            half = s // 2
            up = (rem > half) | ((rem == half) & ((fl & 1) == 1))
            q = fl + up.astype(i32) + woff
            qp = 32 * (col // 32) + 8 * ((col // 4) % 4) + 4 * ((col // 16) % 2) + col % 4
            rep = (q == qp).astype(bf16)
            Rp = _dot(r_hi, rep) + _dot(r_mid, rep) + _dot(r_lo, rep)
            h, l_ = _split2(Rp)
            rhi_s[2 + vi] = h
            rlo_s[2 + vi] = l_

    with jax.named_scope('kprep'):
        T = lambda ref: ref[...].astype(f32).T
        dt = _r(jnp.exp(ldt_ref[...].astype(f32)))
        lam_re = dt * T(are_ref)
        lam_im = dt * T(aim_ref)
        dbr = dt * T(bre_ref)
        dbi = dt * T(bim_ref)
        cr = T(cre_ref)
        ci = T(cim_ref)
        wr = cr * dbr - ci * dbi
        wi = cr * dbi + ci * dbr

        def anchor(k):
            sc = f32(2.0 ** k)
            mag = jnp.exp(lam_re * sc)
            a = lam_im * sc
            return mag * jnp.cos(a), mag * jnp.sin(a)

        def cmul(a, b):
            return a[0] * b[0] - a[1] * b[1], a[0] * b[1] + a[1] * b[0]

        E = []
        for k in range(12):
            if k % 4 == 0:
                E.append(anchor(k))
            else:
                E.append(cmul(E[-1], E[-1]))
        g_s[...] = jnp.zeros_like(g_s)

    cp_x.wait()
    with jax.named_scope('ln'):
        def lnb(i, c):
            r0 = pl.multiple_of(i * MB, MB)
            xn = _ln(x_s[pl.ds(r0, MB), :].astype(f32))
            xn_s[pl.ds(r0, MB), :] = xn.astype(bf16)
            yn_s[pl.ds(r0, MB), :] = _ln(xn).astype(bf16)
            return c
        lax.fori_loop(0, L // MB, lnb, 0)
    cp_w1.wait()
    cp_w2.wait()

    b1 = b1_ref[...].astype(f32)
    b2 = b2_ref[...].astype(f32)

    def mlp_a(c):
        tb = c // 14
        hc = c % 14
        r0 = pl.multiple_of(tb * MB, MB)
        c0 = pl.multiple_of(hc * 128, 128)
        hp = _dot(yn_s[pl.ds(r0, MB), :], w1_s[:, pl.ds(c0, 128)])
        bb_ = b1_ref[:, pl.ds(c0, 128)].astype(f32)
        hp = _r(_r(hp) + bb_)
        h_s[pl.ds(r0, MB), pl.ds(c0, 128)] = jax.nn.gelu(hp, approximate=True).astype(bf16)

    def mlp_b(c):
        tb = c // 4
        oc = c % 4
        r0 = pl.multiple_of(tb * MB, MB)
        c0 = pl.multiple_of(oc * 128, 128)
        yb = _dot(h_s[pl.ds(r0, MB), :], w2_s[:, pl.ds(c0, 128)])
        bb_ = b2_ref[:, pl.ds(c0, 128)].astype(f32)
        yb_s[pl.ds(r0, MB), pl.ds(c0, 128)] = _r(_r(yb) + bb_)

    def build(tr, ti, base, ks):
        tr[0] = base[0]
        ti[0] = base[1]
        for bi, k in enumerate(ks):
            n = 1 << bi
            er, ei = E[k]

            def body(i, c):
                ar = tr[i]
                ai = ti[i]
                tr[i + n] = ar * er - ai * ei
                ti[i + n] = ar * ei + ai * er
                return c
            with jax.named_scope('build'):
                lax.fori_loop(0, n, body, 0)

    def pairs(nbb, row_base, extra):
        def body(idx, c):
            lt = idx % 4
            t = idx // 4
            ab = t // nbb
            bb = t % nbb
            lo = pl.multiple_of(lt * 128, 128)

            def g_body(g, accs):
                off = pl.multiple_of(g * 8, 8)
                xs = [(xr_s[ab * 4 + i, pl.ds(off, 8), pl.ds(lo, 128)],
                       xi_s[ab * 4 + i, pl.ds(off, 8), pl.ds(lo, 128)]) for i in range(4)]
                ys = [(yr_s[bb * 4 + j, pl.ds(off, 8), pl.ds(lo, 128)],
                       yi_s[bb * 4 + j, pl.ds(off, 8), pl.ds(lo, 128)]) for j in range(4)]
                new = []
                for i in range(4):
                    for j in range(4):
                        new.append(accs[i * 4 + j] + (xs[i][0] * ys[j][0] - xs[i][1] * ys[j][1]))
                return tuple(new)

            accs = lax.fori_loop(0, N // 8, g_body,
                                 tuple(jnp.zeros((8, 128), f32) for _ in range(16)), unroll=8)
            for q in range(2):
                row = pl.multiple_of(row_base + t * 16 + q * 8, 8)
                blk8 = jnp.concatenate(
                    [jnp.sum(accs[q * 8 + j], axis=0, keepdims=True) for j in range(8)], axis=0)
                g_s[pl.ds(row, 8), pl.ds(lo, 128)] = blk8
            return c
        with jax.named_scope('pairs'):
            lax.fori_loop(0, 16 * nbb, body, 0)

    w = (wr, wi)
    one = (jnp.ones((N, D), f32), jnp.zeros((N, D), f32))
    build(yr_s, yi_s, one, [0, 1, 2, 3])
    build(xr_s, xi_s, w, [4, 5, 6, 7])
    pairs(4, 0, lambda idx: mlp_a(idx))
    extras = {1: lambda idx: mlp_a(64 + idx),
              2: lambda idx: lax.cond(idx < 16, lambda: mlp_a(96 + idx), lambda: mlp_b(idx - 16)),
              3: lambda idx: mlp_b(16 + idx)}
    for r in (1, 2, 3):
        build(yr_s, yi_s, one, [r, r + 1, r + 2])
        build(xr_s, xi_s, cmul(w, E[7 + r]), [3 + r, 4 + r, 5 + r, 6 + r])
        rb = 256 + (r - 1) * 136
        pairs(2, rb, extras[r])
        endp = cmul(w, E[8 + r])[0]
        g_s[pl.ds(rb + 128, 1), :] = jnp.sum(endp, axis=0, keepdims=True)
    with jax.named_scope('khat'):
        for m in range(NB):
            if m < 2:
                mi, start = 1, 128 * m
            elif m < 4:
                mi, start = 2, 256 + 64 * (m - 2)
            elif m < 8:
                mi, start = 3, 392 + 32 * (m - 4)
            else:
                c = m - 8
                mi, start = 4 + (c % 2), 528 + 32 * (c // 2)
            gm = g_s[pl.ds(start, 128), :]
            gh, gl = _split2(gm)
            kh_s[m] = _dot(rhi_s[mi], gh) + _dot(rhi_s[mi], gl) + _dot(rlo_s[mi], gh)

    krow = lax.broadcasted_iota(i32, (FR, 1), 0)
    kf = jnp.where(krow < RE_ROWS, krow, krow - RE_ROWS)
    sgn = jnp.where(kf % 2 == 0, 1.0, -1.0).astype(f32)

    def fwd(s, uprev):
        row0 = pl.multiple_of(s * P, P)
        xn_b = xn_s[pl.ds(row0, P), :]
        U = _dot(rhi_s[0], xn_b) + _dot(rlo_s[0], xn_b)
        v_s[s] = U + sgn * uprev
        return U
    with jax.named_scope('fwd'):
        lax.fori_loop(0, NB, fwd, jnp.zeros((FR, D), f32))

    def mac(idx, c):
        lt = idx % 4
        g = idx // 4
        lanes = pl.ds(pl.multiple_of(lt * 128, 128), 128)
        rr = pl.ds(pl.multiple_of(g * 8, 8), 8)
        ri = pl.ds(pl.multiple_of(RE_ROWS + g * 8, 8), 8)
        Kr = [kh_s[m, rr, lanes] for m in range(NB)]
        Ki = [kh_s[m, ri, lanes] for m in range(NB)]
        for s0 in range(0, NB, 2):
            ar0 = ai0 = ar1 = ai1 = None
            for i in range(s0 + 2):
                vr = v_s[i, rr, lanes]
                vi = v_s[i, ri, lanes]
                if i <= s0:
                    m = s0 - i
                    tr_ = Kr[m] * vr - Ki[m] * vi
                    ti_ = Kr[m] * vi + Ki[m] * vr
                    ar0 = tr_ if ar0 is None else ar0 + tr_
                    ai0 = ti_ if ai0 is None else ai0 + ti_
                m = s0 + 1 - i
                tr_ = Kr[m] * vr - Ki[m] * vi
                ti_ = Kr[m] * vi + Ki[m] * vr
                ar1 = tr_ if ar1 is None else ar1 + tr_
                ai1 = ti_ if ai1 is None else ai1 + ti_
            w_s[s0, rr, lanes] = ar0
            w_s[s0, ri, lanes] = ai0
            w_s[s0 + 1, rr, lanes] = ar1
            w_s[s0 + 1, ri, lanes] = ai1
        return c

    with jax.named_scope('mac'):
        lax.fori_loop(0, 64, mac, 0)
        ny = pl.ds(P, 8)
        for s in range(NB):
            acc = None
            for m in range(s + 1):
                t_ = kh_s[m, ny, :] * v_s[s - m, ny, :]
                acc = t_ if acc is None else acc + t_
            w_s[s, ny, :] = acc

    dsk = dsk_ref[...].astype(f32)

    def blk(sb, c):
        row0 = pl.multiple_of(sb * MB, MB)
        xf = x_s[pl.ds(row0, MB), :].astype(f32)
        xn = xn_s[pl.ds(row0, MB), :].astype(f32)
        ys = []
        for h in range(MB // P):
            W = w_s[sb * (MB // P) + h]
            wh, wl = _split2(W)
            ys.append(_dot(ihi_s[...], wh) + _dot(ihi_s[...], wl) + _dot(ilo_s[...], wh))
        y = jnp.concatenate(ys, axis=0)
        yA = _r(_r(y) + _r(xn * dsk))
        yn = yn_s[pl.ds(row0, MB), :]
        hp = _r(_r(_dot(yn, w1_s[...])) + b1)
        hg = jax.nn.gelu(hp, approximate=True).astype(bf16)
        yB = _r(_r(_dot(hg, w2_s[...])) + b2)
        o_s[pl.ds(row0, MB), :] = (_r(xf + yA) + yB).astype(bf16)
        pltpu.make_async_copy(o_s.at[pl.ds(row0, MB), :], o_hbm.at[pl.ds(row0, MB), :], sems.at[3]).start()
        return c

    with jax.named_scope('main'):
        lax.fori_loop(0, L // MB, blk, 0)
    pltpu.make_async_copy(o_s, o_hbm, sems.at[3]).wait()


@jax.jit
def pallas_parallel_sum__ssm_conv_s4__mixer_channel_mlp__prompt_kernel(A_u, A_A_re, A_A_im, A_B_re, A_B_im, A_C_re, A_C_im, A_log_dt, A_Dskip, B_x, B_w1, B_b1, B_w2, B_b2):
    x = A_u.reshape(L, D)
    anyspec = pl.BlockSpec(memory_space=pl.ANY)
    vm = pl.BlockSpec(memory_space=pltpu.VMEM)
    out = pl.pallas_call(
        kernel,
        out_shape=jax.ShapeDtypeStruct((L, D), bf16),
        in_specs=[anyspec, vm, vm, vm, vm, vm, vm, vm, vm, anyspec, vm, anyspec, vm],
        out_specs=anyspec,
        scratch_shapes=[
            pltpu.VMEM((16, N, D), f32), pltpu.VMEM((16, N, D), f32),
            pltpu.VMEM((16, N, D), f32), pltpu.VMEM((16, N, D), f32),
            pltpu.VMEM((768, D), f32),
            pltpu.VMEM((NB, FR, D), f32),
            pltpu.VMEM((NB, FR, D), f32),
            pltpu.VMEM((6, FR, P), bf16), pltpu.VMEM((6, FR, P), bf16),
            pltpu.VMEM((P, FR), bf16), pltpu.VMEM((P, FR), bf16),
            pltpu.VMEM((L, D), bf16),
            pltpu.VMEM((NB, FR, D), f32),
            pltpu.VMEM((L, D), bf16),
            pltpu.VMEM((D, F), bf16),
            pltpu.VMEM((F, D), bf16),
            pltpu.VMEM((L, D), bf16),
            pltpu.VMEM((L, F), bf16),
            pltpu.VMEM((L, D), f32),
            pltpu.VMEM((L, D), bf16),
            pltpu.SemaphoreType.DMA((4,)),
        ],
        compiler_params=pltpu.CompilerParams(vmem_limit_bytes=110 * 1024 * 1024),
    )(x, A_A_re, A_A_im, A_B_re, A_B_im, A_C_re, A_C_im,
      A_log_dt.reshape(1, D), A_Dskip.reshape(1, D),
      B_w1, B_b1.reshape(1, F), B_w2, B_b2.reshape(1, D))
    return out.reshape(1, L, D)
```

```python
import functools
import numpy as np
import jax
import jax.numpy as jnp
from jax import lax
import jax.experimental.pallas as pl
import jax.experimental.pallas.tpu as pltpu

f32 = jnp.float32
bf16 = jnp.bfloat16
i32 = jnp.int32

L = 2048
D = 512
N = 128
F = 1792
P = 128
NB = L // P
FR = 264
RE_ROWS = 136
MB = 256
MERGE = False


def _r(x):
    return x.astype(bf16).astype(f32)


def _ln(xf):
    mean = jnp.mean(xf, axis=-1, keepdims=True)
    cen = xf - mean
    var = jnp.mean(cen * cen, axis=-1, keepdims=True)
    m_b = _r(mean)
    v_b = _r(var)
    d = _r(xf - m_b)
    den = _r(jnp.sqrt(_r(v_b + 1e-5)))
    return _r(d / den)


def _split2(a):
    hi = a.astype(bf16)
    lo = (a - hi.astype(f32)).astype(bf16)
    return hi, lo


def _dot(a, b):
    return jnp.dot(a, b, preferred_element_type=f32)


def _dft_rows(delta):
    kk = lax.broadcasted_iota(i32, (FR, P), 0)
    is_re = kk < RE_ROWS
    kfreq = jnp.where(is_re, kk, kk - RE_ROWS)
    valid = jnp.logical_or(jnp.logical_not(is_re), kk <= P)
    ang = ((kfreq * delta) % (2 * P)).astype(f32) * f32(np.pi / P)
    Rm = jnp.where(is_re, jnp.cos(ang), -jnp.sin(ang))
    return jnp.where(valid, Rm, 0.0)


def kernel(x_hbm, are_ref, aim_ref, bre_ref, bim_ref, cre_ref, cim_ref, ldt_ref, dsk_ref,
           w1_hbm, b1_ref, w2_hbm, b2_ref, o_hbm,
           xr_s, xi_s, yr_s, yi_s, g_s, kh_s, v_s, rhi_s, rlo_s, ihi_s, ilo_s, xn_s, w_s,
           x_s, w1_s, w2_s, yn_s, h_s, yb_s, o_s, sems):
    cp_x = pltpu.make_async_copy(x_hbm, x_s, sems.at[0])
    cp_w1 = pltpu.make_async_copy(w1_hbm, w1_s, sems.at[1])
    cp_w2 = pltpu.make_async_copy(w2_hbm, w2_s, sems.at[2])
    cp_x.start()
    cp_w1.start()
    cp_w2.start()

    with jax.named_scope('dftmat'):
        jj = lax.broadcasted_iota(i32, (FR, P), 1)
        Rm = _dft_rows(jj)
        ii = lax.broadcasted_iota(i32, (P, FR), 0)
        kc = lax.broadcasted_iota(i32, (P, FR), 1)
        c_re = kc < RE_ROWS
        kf2 = jnp.where(c_re, kc, kc - RE_ROWS)
        ang2 = ((kf2 * ii) % (2 * P)).astype(f32) * f32(np.pi / P)
        wgt = jnp.where((kf2 == 0) | (kf2 == P), 1.0, 2.0) * f32(1.0 / (2 * P))
        valid2 = jnp.logical_or(jnp.logical_not(c_re), kc <= P)
        Im = jnp.where(c_re, jnp.cos(ang2), -jnp.sin(ang2)) * wgt
        Im = jnp.where(valid2, Im, 0.0)
        ih, il = _split2(Im)
        ihi_s[...] = ih
        ilo_s[...] = il
        h, l_ = _split2(Rm)
        rhi_s[0] = h
        rlo_s[0] = l_
        rho = jj
        delta_near = 64 * (rho // 64) + 16 * ((rho // 4) % 4) + 4 * ((rho // 16) % 4) + rho % 4
        h, l_ = _split2(_dft_rows(delta_near))
        rhi_s[1] = h
        rlo_s[1] = l_
        r_hi = Rm.astype(bf16)
        rem1 = Rm - r_hi.astype(f32)
        r_mid = rem1.astype(bf16)
        r_lo = (rem1 - r_mid.astype(f32)).astype(bf16)
        dl = lax.broadcasted_iota(i32, (P, P), 0)
        col = lax.broadcasted_iota(i32, (P, P), 1)
        for vi, (r, woff) in enumerate([(1, 0), (2, 0), (3, 0), (3, 8)]):
            s = 1 << r
            fl = dl >> r
            rem = dl & (s - 1)
            half = s // 2
            up = (rem > half) | ((rem == half) & ((fl & 1) == 1))
            q = fl + up.astype(i32) + woff
            qp = 32 * (col // 32) + 8 * ((col // 4) % 4) + 4 * ((col // 16) % 2) + col % 4
            rep = (q == qp).astype(bf16)
            Rp = _dot(r_hi, rep) + _dot(r_mid, rep) + _dot(r_lo, rep)
            h, l_ = _split2(Rp)
            rhi_s[2 + vi] = h
            rlo_s[2 + vi] = l_

    with jax.named_scope('kprep'):
        T = lambda ref: ref[...].astype(f32).T
        dt = _r(jnp.exp(ldt_ref[...].reshape(1, D).astype(f32)))
        lam_re = dt * T(are_ref)
        lam_im = dt * T(aim_ref)
        dbr = dt * T(bre_ref)
        dbi = dt * T(bim_ref)
        cr = T(cre_ref)
        ci = T(cim_ref)
        wr = cr * dbr - ci * dbi
        wi = cr * dbi + ci * dbr

        def anchor(k):
            sc = f32(2.0 ** k)
            mag = jnp.exp(lam_re * sc)
            a = lam_im * sc
            return mag * jnp.cos(a), mag * jnp.sin(a)

        def cmul(a, b):
            return a[0] * b[0] - a[1] * b[1], a[0] * b[1] + a[1] * b[0]

        E = []
        for k in range(12):
            if k % 4 == 0:
                E.append(anchor(k))
            else:
                E.append(cmul(E[-1], E[-1]))
        g_s[...] = jnp.zeros_like(g_s)

    cp_x.wait()
    with jax.named_scope('ln'):
        def lnb(i, c):
            r0 = pl.multiple_of(i * MB, MB)
            xn = _ln(x_s[pl.ds(r0, MB), :].astype(f32))
            xn_s[pl.ds(r0, MB), :] = xn.astype(bf16)
            yn_s[pl.ds(r0, MB), :] = _ln(xn).astype(bf16)
            return c
        lax.fori_loop(0, L // MB, lnb, 0)
    cp_w1.wait()
    cp_w2.wait()

    b1 = b1_ref[...].reshape(1, F).astype(f32)
    b2 = b2_ref[...].reshape(1, D).astype(f32)

    def build(tr, ti, base, ks):
        tr[0] = base[0]
        ti[0] = base[1]
        for bi, k in enumerate(ks):
            n = 1 << bi
            er, ei = E[k]

            def body(i, c):
                ar = tr[i]
                ai = ti[i]
                tr[i + n] = ar * er - ai * ei
                ti[i + n] = ar * ei + ai * er
                return c
            with jax.named_scope('build'):
                lax.fori_loop(0, n, body, 0)

    def pairs(nbb, row_base, extra):
        def body(idx, c):
            lt = idx % 4
            t = idx // 4
            ab = t // nbb
            bb = t % nbb
            lo = pl.multiple_of(lt * 128, 128)

            def g_body(g, accs):
                off = pl.multiple_of(g * 8, 8)
                xs = [(xr_s[ab * 4 + i, pl.ds(off, 8), pl.ds(lo, 128)],
                       xi_s[ab * 4 + i, pl.ds(off, 8), pl.ds(lo, 128)]) for i in range(4)]
                ys = [(yr_s[bb * 4 + j, pl.ds(off, 8), pl.ds(lo, 128)],
                       yi_s[bb * 4 + j, pl.ds(off, 8), pl.ds(lo, 128)]) for j in range(4)]
                new = []
                for i in range(4):
                    for j in range(4):
                        new.append(accs[i * 4 + j] + (xs[i][0] * ys[j][0] - xs[i][1] * ys[j][1]))
                return tuple(new)

            accs = lax.fori_loop(0, N // 8, g_body,
                                 tuple(jnp.zeros((8, 128), f32) for _ in range(16)), unroll=8)
            for q in range(2):
                row = pl.multiple_of(row_base + t * 16 + q * 8, 8)
                blk8 = jnp.concatenate(
                    [jnp.sum(accs[q * 8 + j], axis=0, keepdims=True) for j in range(8)], axis=0)
                g_s[pl.ds(row, 8), pl.ds(lo, 128)] = blk8
            return c
        with jax.named_scope('pairs'):
            lax.fori_loop(0, 16 * nbb, body, 0)

    w = (wr, wi)
    one = (jnp.ones((N, D), f32), jnp.zeros((N, D), f32))
    build(yr_s, yi_s, one, [0, 1, 2, 3])
    build(xr_s, xi_s, w, [4, 5, 6, 7])
    pairs(4, 0, lambda idx: mlp_a(idx))
    extras = {1: lambda idx: mlp_a(64 + idx),
              2: lambda idx: lax.cond(idx < 16, lambda: mlp_a(96 + idx), lambda: mlp_b(idx - 16)),
              3: lambda idx: mlp_b(16 + idx)}
    for r in (1, 2, 3):
        build(yr_s, yi_s, one, [r, r + 1, r + 2])
        build(xr_s, xi_s, cmul(w, E[7 + r]), [3 + r, 4 + r, 5 + r, 6 + r])
        rb = 256 + (r - 1) * 136
        pairs(2, rb, extras[r])
        endp = cmul(w, E[8 + r])[0]
        g_s[pl.ds(rb + 128, 1), :] = jnp.sum(endp, axis=0, keepdims=True)
    with jax.named_scope('khat'):
        for m in range(NB):
            if m < 2:
                mi, start = 1, 128 * m
            elif m < 4:
                mi, start = 2, 256 + 64 * (m - 2)
            elif m < 8:
                mi, start = 3, 392 + 32 * (m - 4)
            else:
                c = m - 8
                mi, start = 4 + (c % 2), 528 + 32 * (c // 2)
            gm = g_s[pl.ds(start, 128), :]
            gh, gl = _split2(gm)
            kh_s[m] = _dot(rhi_s[mi], gh) + _dot(rhi_s[mi], gl) + _dot(rlo_s[mi], gh)

    krow = lax.broadcasted_iota(i32, (FR, 1), 0)
    kf = jnp.where(krow < RE_ROWS, krow, krow - RE_ROWS)
    sgn = jnp.where(kf % 2 == 0, 1.0, -1.0).astype(f32)

    def fwd(s, uprev):
        row0 = pl.multiple_of(s * P, P)
        xn_b = xn_s[pl.ds(row0, P), :]
        U = _dot(rhi_s[0], xn_b) + _dot(rlo_s[0], xn_b)
        v_s[s] = U + sgn * uprev
        return U
    with jax.named_scope('fwd'):
        lax.fori_loop(0, NB, fwd, jnp.zeros((FR, D), f32))

    def mac(idx, c):
        lt = idx % 4
        g = idx // 4
        lanes = pl.ds(pl.multiple_of(lt * 128, 128), 128)
        rr = pl.ds(pl.multiple_of(g * 8, 8), 8)
        ri = pl.ds(pl.multiple_of(RE_ROWS + g * 8, 8), 8)
        Kr = [kh_s[m, rr, lanes] for m in range(NB)]
        Ki = [kh_s[m, ri, lanes] for m in range(NB)]
        for s0 in range(0, NB, 2):
            ar0 = ai0 = ar1 = ai1 = None
            for i in range(s0 + 2):
                vr = v_s[i, rr, lanes]
                vi = v_s[i, ri, lanes]
                if i <= s0:
                    m = s0 - i
                    tr_ = Kr[m] * vr - Ki[m] * vi
                    ti_ = Kr[m] * vi + Ki[m] * vr
                    ar0 = tr_ if ar0 is None else ar0 + tr_
                    ai0 = ti_ if ai0 is None else ai0 + ti_
                m = s0 + 1 - i
                tr_ = Kr[m] * vr - Ki[m] * vi
                ti_ = Kr[m] * vi + Ki[m] * vr
                ar1 = tr_ if ar1 is None else ar1 + tr_
                ai1 = ti_ if ai1 is None else ai1 + ti_
            w_s[s0, rr, lanes] = ar0
            w_s[s0, ri, lanes] = ai0
            w_s[s0 + 1, rr, lanes] = ar1
            w_s[s0 + 1, ri, lanes] = ai1
        return c

    with jax.named_scope('mac'):
        lax.fori_loop(0, 64, mac, 0)
        ny = pl.ds(P, 8)
        for s in range(NB):
            acc = None
            for m in range(s + 1):
                t_ = kh_s[m, ny, :] * v_s[s - m, ny, :]
                acc = t_ if acc is None else acc + t_
            w_s[s, ny, :] = acc

    dsk = dsk_ref[...].reshape(1, D).astype(f32)

    def blk(sb, c):
        row0 = pl.multiple_of(sb * MB, MB)
        xf = x_s[pl.ds(row0, MB), :].astype(f32)
        xn = xn_s[pl.ds(row0, MB), :].astype(f32)
        ys = []
        for h in range(MB // P):
            W = w_s[sb * (MB // P) + h]
            wh, wl = _split2(W)
            ys.append(_dot(ihi_s[...], wh) + _dot(ihi_s[...], wl) + _dot(ilo_s[...], wh))
        y = jnp.concatenate(ys, axis=0)
        yA = _r(_r(y) + _r(xn * dsk))
        yn = yn_s[pl.ds(row0, MB), :]
        hp = _r(_r(_dot(yn, w1_s[...])) + b1)
        hg = jax.nn.gelu(hp, approximate=True).astype(bf16)
        yB = _r(_r(_dot(hg, w2_s[...])) + b2)
        o_s[pl.ds(row0, MB), :] = (_r(xf + yA) + yB).astype(bf16)
        pltpu.make_async_copy(o_s.at[pl.ds(row0, MB), :], o_hbm.at[pl.ds(row0, MB), :], sems.at[3]).start()
        return c

    with jax.named_scope('main'):
        lax.fori_loop(0, L // MB, blk, 0)
    pltpu.make_async_copy(o_s, o_hbm, sems.at[3]).wait()


@jax.jit
def pallas_parallel_sum__ssm_conv_s4__mixer_channel_mlp__prompt_kernel(A_u, A_A_re, A_A_im, A_B_re, A_B_im, A_C_re, A_C_im, A_log_dt, A_Dskip, B_x, B_w1, B_b1, B_w2, B_b2):
    x = A_u.reshape(L, D)
    anyspec = pl.BlockSpec(memory_space=pl.ANY)
    vm = pl.BlockSpec(memory_space=pltpu.VMEM)
    out = pl.pallas_call(
        kernel,
        out_shape=jax.ShapeDtypeStruct((L, D), bf16),
        in_specs=[anyspec, vm, vm, vm, vm, vm, vm, vm, vm, anyspec, vm, anyspec, vm],
        out_specs=anyspec,
        scratch_shapes=[
            pltpu.VMEM((16, N, D), f32), pltpu.VMEM((16, N, D), f32),
            pltpu.VMEM((16, N, D), f32), pltpu.VMEM((16, N, D), f32),
            pltpu.VMEM((768, D), f32),
            pltpu.VMEM((NB, FR, D), f32),
            pltpu.VMEM((NB, FR, D), f32),
            pltpu.VMEM((6, FR, P), bf16), pltpu.VMEM((6, FR, P), bf16),
            pltpu.VMEM((P, FR), bf16), pltpu.VMEM((P, FR), bf16),
            pltpu.VMEM((L, D), bf16),
            pltpu.VMEM((NB, FR, D), f32),
            pltpu.VMEM((L, D), bf16),
            pltpu.VMEM((D, F), bf16),
            pltpu.VMEM((F, D), bf16),
            pltpu.VMEM((L, D), bf16),
            pltpu.VMEM((L, F), bf16),
            pltpu.VMEM((L, D), f32),
            pltpu.VMEM((L, D), bf16),
            pltpu.SemaphoreType.DMA((4,)),
        ],
        compiler_params=pltpu.CompilerParams(vmem_limit_bytes=110 * 1024 * 1024),
    )(x, A_A_re, A_A_im, A_B_re, A_B_im, A_C_re, A_C_im,
      A_log_dt, A_Dskip,
      B_w1, B_b1, B_w2, B_b2)
    return out.reshape(1, L, D)
```
